```python
import os as _os
_os.environ.setdefault("JAX_PLATFORMS", "cpu")
import jax
import jax.numpy as jnp

def _softmax(x, axis=-1):
    return jax.nn.softmax(x, axis=axis)
def _gelu(x):
    return jax.nn.gelu(x, approximate=True)
def _silu(x):
    return jax.nn.silu(x)
def _sigmoid(x):
    return jax.nn.sigmoid(x)
def _layernorm(x, axis=-1, eps=1e-5):
    m = jnp.mean(x, axis=axis, keepdims=True)
    v = jnp.var(x, axis=axis, keepdims=True)
    return (x - m) / jnp.sqrt(v + eps)
def _scatter_add(tgt, idx, src, axis=0):
    return tgt.at[idx].add(src)
def _segment_sum(src, seg, n):
    return jax.ops.segment_sum(src, seg, n)
class _Rng:
    def __init__(self, key):
        self._k = key
    def _next(self):
        self._k, sub = jax.random.split(self._k)
        return sub
    def normal(self, shape):
        return jax.random.normal(self._next(), shape, dtype=jnp.bfloat16)
    def randint(self, lo, hi, shape):
        return jax.random.randint(self._next(), shape, lo, hi, dtype=jnp.int32)
    def uniform(self, shape, lo=0.0, hi=1.0):
        return jax.random.uniform(self._next(), shape, jnp.bfloat16, lo, hi)
    def permutation(self, n):
        return jax.random.permutation(self._next(), n)


kernel_name = 'standalone__linear_kernel_rfa__decode'

def setup_inputs():
    _rng = _Rng(jax.random.key(int.from_bytes(__import__("os").urandom(4), "little")))
    _w = (lambda a: (lambda t: t.astype(jnp.bfloat16) if jnp.issubdtype(t.dtype, jnp.floating) else t)(jnp.asarray(a)))
    B, H, Sq, Sk, D, M = 2, 16, 1, 16384, 256, 16
    return {
        "q": _w((lambda *s: _rng.normal(s) * 0.4)(B, H, Sq, D)),
        "k": _w((lambda *s: _rng.normal(s) * 1.6)(B, H, Sk, D)),
        "v": _w((lambda *s: _rng.normal(s) * 1.6)(B, H, Sk, D)),
        "omega": _w((lambda *s: _rng.normal(s) * 1.6)(M, D)),
    }

def reference(q, k, v, omega):
    d = q.shape[-1]
    m = omega.shape[0]
    scale = float(d) ** -0.25
    qs = q * scale
    ks = k * scale
    q_proj = jnp.einsum("bhsd,md->bhsm", qs, omega)
    k_proj = jnp.einsum("bhsd,md->bhsm", ks, omega)
    q_sq = 0.5 * jnp.einsum("bhsd,bhsd->bhs", qs, qs)[..., None]
    k_sq = 0.5 * jnp.einsum("bhsd,bhsd->bhs", ks, ks)[..., None]
    inv_sqrt_m = float(m) ** -0.5
    phi_q = jnp.exp(q_proj - q_sq) * inv_sqrt_m + 1e-6
    phi_k = jnp.exp(k_proj - k_sq) * inv_sqrt_m + 1e-6
    kv = jnp.einsum("bhsm,bhsd->bhmd", phi_k, v)
    z  = jnp.einsum("bhsm->bhm", phi_k)
    num = jnp.einsum("bhqm,bhmd->bhqd", phi_q, kv)
    den = jnp.einsum("bhqm,bhm->bhq", phi_q, z)[..., None] + 1e-6
    return num / den
```

```python
import functools

import jax
import jax.numpy as jnp
import jax.experimental.pallas as pl
import jax.experimental.pallas.tpu as pltpu

F32, BF16 = jnp.float32, jnp.bfloat16
_NT = (((1,), (1,)), ((), ()))
_EPS = 9.98377799987793e-07

_TC = 512
_NB = 8
_CR = 64
_PATTERN = ((0, 0, 0), (0, 2, 1), (0, 1, 0), (0, 3, 1),
            (1, 0, 0), (1, 2, 1), (1, 1, 0), (1, 3, 1))
_GROUP = 4 * _CR


def _r(x):
    return x.astype(BF16).astype(F32)


def _split(s):
    hi = s.astype(BF16)
    return hi, (s - hi.astype(F32)).astype(BF16)


def _kernel(q_ref, om_ref, k_hbm, v_hbm, o_ref, kb, vb, of_ref, sem, *, sk):
    bh, d = q_ref.shape
    m = om_ref.shape[0]
    n_tiles = k_hbm.shape[0] // _TC
    tiles_per_head = sk // _TC
    scale = float(d) ** -0.25
    inv_sqrt_m = float(m) ** -0.5
    half = d // 2

    def start(t, slot):
        for g in range(_TC // _GROUP):
            for a, c, prio in _PATTERN:
                src, dst = ((k_hbm, kb), (v_hbm, vb))[a]
                off = g * _GROUP + c * _CR
                pltpu.make_async_copy(
                    src.at[pl.ds(t * _TC + off, _CR)],
                    dst.at[slot, pl.ds(off, _CR)],
                    sem.at[a, slot],
                ).start(priority=prio)

    def wait(slot):
        pltpu.make_async_copy(kb.at[slot], kb.at[slot], sem.at[0, slot]).wait()
        pltpu.make_async_copy(vb.at[slot], vb.at[slot], sem.at[1, slot]).wait()

    for i in range(_NB - 1):
        start(i, i)

    om = om_ref[...]
    ones = jnp.ones((8, d), BF16)

    def features(proj, sq):
        x = _r(_r(proj) - 0.5 * _r(sq))
        return _r(_r(jnp.exp(x)) * inv_sqrt_m + _EPS)

    qs = (q_ref[...].astype(F32) * scale).astype(BF16)
    qf = qs.astype(F32)
    q_hi, q_lo = _split(qf * qf)
    q_sq = (jax.lax.dot_general(ones, q_hi, _NT, preferred_element_type=F32)
            + jax.lax.dot_general(ones, q_lo, _NT, preferred_element_type=F32))[0:1]
    phi_q = features(jax.lax.dot_general(om, qs, _NT, preferred_element_type=F32), q_sq)
    lane = jax.lax.broadcasted_iota(jnp.int32, phi_q.shape, 1)

    def head(h, _):
        def tile(j, carry):
            acc, zacc = carry
            t = h * tiles_per_head + j
            nt = t + _NB - 1

            @pl.when(nt < n_tiles)
            def _():
                start(nt, nt % _NB)

            slot = t % _NB
            wait(slot)
            k = kb[slot]
            k_proj = jax.lax.dot_general(om, k, _NT, preferred_element_type=F32) * scale
            kf = k.astype(F32)
            s = kf[:, :half] * kf[:, :half] + kf[:, half:] * kf[:, half:]
            k_sq = jax.lax.dot_general(
                ones, jnp.concatenate(_split(s), axis=1), _NT, preferred_element_type=F32
            )[0:1] * (scale * scale)
            phi = features(k_proj, k_sq)
            acc = acc + jnp.dot(phi.astype(BF16), vb[slot], preferred_element_type=F32)
            for i in range(_TC // 128):
                zacc = zacc + phi[:, i * 128:(i + 1) * 128]
            return acc, zacc

        acc, zacc = jax.lax.fori_loop(
            0, tiles_per_head, tile, (jnp.zeros((m, d), F32), jnp.zeros((m, 128), F32)))
        pq = jnp.sum(jnp.where(lane == h, phi_q, 0.0), axis=1, keepdims=True)
        num = _r(jnp.sum(pq * _r(acc), axis=0, keepdims=True))
        z = _r(jnp.sum(zacc, axis=1, keepdims=True))
        den = _r(_r(jnp.sum(pq * z, axis=0, keepdims=True)) + _EPS)
        of_ref[pl.ds(h, 1), :] = num / den
        return 0

    jax.lax.fori_loop(0, bh, head, 0)
    o_ref[...] = of_ref[...].astype(o_ref.dtype)


@jax.jit
def pallas_standalone__linear_kernel_rfa__decode_kernel(
    q: jax.Array,
    k: jax.Array,
    v: jax.Array,
    omega: jax.Array,
):
    B, H, Sq, D = q.shape
    Sk = k.shape[2]
    assert Sq == 1 and Sk % _TC == 0 and B * H * Sk // _TC >= _NB
    out = pl.pallas_call(
        functools.partial(_kernel, sk=Sk),
        in_specs=[
            pl.BlockSpec(memory_space=pltpu.VMEM),
            pl.BlockSpec(memory_space=pltpu.VMEM),
            pl.BlockSpec(memory_space=pl.ANY),
            pl.BlockSpec(memory_space=pl.ANY),
        ],
        out_specs=pl.BlockSpec(memory_space=pltpu.VMEM),
        out_shape=jax.ShapeDtypeStruct((B * H, D), q.dtype),
        scratch_shapes=[
            pltpu.VMEM((_NB, _TC, D), BF16),
            pltpu.VMEM((_NB, _TC, D), BF16),
            pltpu.VMEM((B * H, D), F32),
            pltpu.SemaphoreType.DMA((2, _NB)),
        ],
        compiler_params=pltpu.CompilerParams(vmem_limit_bytes=64 * 2**20),
    )(q.reshape(B * H, D), omega, k.reshape(B * H * Sk, D), v.reshape(B * H * Sk, D))
    return out.reshape(B, H, Sq, D)
```

```python
import functools

import jax
import jax.numpy as jnp
import jax.experimental.pallas as pl
import jax.experimental.pallas.tpu as pltpu

F32, BF16 = jnp.float32, jnp.bfloat16
_NT = (((1,), (1,)), ((), ()))
_EPS = 9.98377799987793e-07

_TC = 512
_NB = 7
_CR = 64
_PATTERN = ((0, 0, 0), (0, 6, 1), (0, 1, 0), (0, 7, 1),
            (1, 0, 0), (1, 6, 1), (1, 1, 0), (1, 7, 1),
            (0, 4, 0), (0, 2, 1), (0, 5, 0), (0, 3, 1),
            (1, 4, 0), (1, 2, 1), (1, 5, 0), (1, 3, 1))
_GROUP = 8 * _CR


def _r(x):
    return x.astype(BF16).astype(F32)


def _split(s):
    hi = s.astype(BF16)
    return hi, (s - hi.astype(F32)).astype(BF16)


def _kernel(q_ref, om_ref, k_hbm, v_hbm, o_ref, kb, vb, of_ref, sem, *, sk):
    bh, d = q_ref.shape
    m = om_ref.shape[0]
    n_tiles = k_hbm.shape[0] // _TC
    tiles_per_head = sk // _TC
    scale = float(d) ** -0.25
    inv_sqrt_m = float(m) ** -0.5
    half = d // 2

    def start(t, slot):
        for g in range(_TC // _GROUP):
            for a, c, prio in _PATTERN:
                src, dst = ((k_hbm, kb), (v_hbm, vb))[a]
                off = g * _GROUP + c * _CR
                pltpu.make_async_copy(
                    src.at[pl.ds(t * _TC + off, _CR)],
                    dst.at[slot, pl.ds(off, _CR)],
                    sem.at[a, slot],
                ).start(priority=prio)

    def wait(slot):
        pltpu.make_async_copy(kb.at[slot], kb.at[slot], sem.at[0, slot]).wait()
        pltpu.make_async_copy(vb.at[slot], vb.at[slot], sem.at[1, slot]).wait()

    for i in range(_NB - 1):
        start(i, i)

    om = om_ref[...]
    ones = jnp.ones((8, d), BF16)

    def features(proj, sq):
        x = _r(_r(proj) - 0.5 * _r(sq))
        return _r(_r(jnp.exp(x)) * inv_sqrt_m + _EPS)

    qs = (q_ref[...].astype(F32) * scale).astype(BF16)
    qf = qs.astype(F32)
    q_hi, q_lo = _split(qf * qf)
    q_sq = (jax.lax.dot_general(ones, q_hi, _NT, preferred_element_type=F32)
            + jax.lax.dot_general(ones, q_lo, _NT, preferred_element_type=F32))[0:1]
    phi_q = features(jax.lax.dot_general(om, qs, _NT, preferred_element_type=F32), q_sq)
    lane = jax.lax.broadcasted_iota(jnp.int32, phi_q.shape, 1)

    def head(h, _):
        def tile(j, carry):
            acc, zacc = carry
            t = h * tiles_per_head + j
            nt = t + _NB - 1

            @pl.when(nt < n_tiles)
            def _():
                start(nt, nt % _NB)

            slot = t % _NB
            wait(slot)
            k = kb[slot]
            k_proj = jax.lax.dot_general(om, k, _NT, preferred_element_type=F32) * scale
            kf = k.astype(F32)
            s = kf[:, :half] * kf[:, :half] + kf[:, half:] * kf[:, half:]
            k_sq = jax.lax.dot_general(
                ones, jnp.concatenate(_split(s), axis=1), _NT, preferred_element_type=F32
            )[0:1] * (scale * scale)
            phi = features(k_proj, k_sq)
            acc = acc + jnp.dot(phi.astype(BF16), vb[slot], preferred_element_type=F32)
            for i in range(_TC // 128):
                zacc = zacc + phi[:, i * 128:(i + 1) * 128]
            return acc, zacc

        acc, zacc = jax.lax.fori_loop(
            0, tiles_per_head, tile, (jnp.zeros((m, d), F32), jnp.zeros((m, 128), F32)))
        pq = jnp.sum(jnp.where(lane == h, phi_q, 0.0), axis=1, keepdims=True)
        num = _r(jnp.sum(pq * _r(acc), axis=0, keepdims=True))
        z = _r(jnp.sum(zacc, axis=1, keepdims=True))
        den = _r(_r(jnp.sum(pq * z, axis=0, keepdims=True)) + _EPS)
        of_ref[pl.ds(h, 1), :] = num / den
        return 0

    jax.lax.fori_loop(0, bh, head, 0)
    o_ref[...] = of_ref[...].astype(o_ref.dtype)


@jax.jit
def pallas_standalone__linear_kernel_rfa__decode_kernel(
    q: jax.Array,
    k: jax.Array,
    v: jax.Array,
    omega: jax.Array,
):
    B, H, Sq, D = q.shape
    Sk = k.shape[2]
    assert Sq == 1 and Sk % _TC == 0 and B * H * Sk // _TC >= _NB
    out = pl.pallas_call(
        functools.partial(_kernel, sk=Sk),
        in_specs=[
            pl.BlockSpec(memory_space=pltpu.VMEM),
            pl.BlockSpec(memory_space=pltpu.VMEM),
            pl.BlockSpec(memory_space=pl.ANY),
            pl.BlockSpec(memory_space=pl.ANY),
        ],
        out_specs=pl.BlockSpec(memory_space=pltpu.VMEM),
        out_shape=jax.ShapeDtypeStruct((B * H, D), q.dtype),
        scratch_shapes=[
            pltpu.VMEM((_NB, _TC, D), BF16),
            pltpu.VMEM((_NB, _TC, D), BF16),
            pltpu.VMEM((B * H, D), F32),
            pltpu.SemaphoreType.DMA((2, _NB)),
        ],
        compiler_params=pltpu.CompilerParams(vmem_limit_bytes=64 * 2**20),
    )(q.reshape(B * H, D), omega, k.reshape(B * H * Sk, D), v.reshape(B * H * Sk, D))
    return out.reshape(B, H, Sq, D)
```
